```python
import os as _os
_os.environ.setdefault("JAX_PLATFORMS", "cpu")
import jax
import jax.numpy as jnp

def _softmax(x, axis=-1):
    return jax.nn.softmax(x, axis=axis)
def _gelu(x):
    return jax.nn.gelu(x, approximate=True)
def _silu(x):
    return jax.nn.silu(x)
def _sigmoid(x):
    return jax.nn.sigmoid(x)
def _layernorm(x, axis=-1, eps=1e-5):
    m = jnp.mean(x, axis=axis, keepdims=True)
    v = jnp.var(x, axis=axis, keepdims=True)
    return (x - m) / jnp.sqrt(v + eps)
def _scatter_add(tgt, idx, src, axis=0):
    return tgt.at[idx].add(src)
def _segment_sum(src, seg, n):
    return jax.ops.segment_sum(src, seg, n)
class _Rng:
    def __init__(self, key):
        self._k = key
    def _next(self):
        self._k, sub = jax.random.split(self._k)
        return sub
    def normal(self, shape):
        return jax.random.normal(self._next(), shape, dtype=jnp.bfloat16)
    def randint(self, lo, hi, shape):
        return jax.random.randint(self._next(), shape, lo, hi, dtype=jnp.int32)
    def uniform(self, shape, lo=0.0, hi=1.0):
        return jax.random.uniform(self._next(), shape, jnp.bfloat16, lo, hi)
    def permutation(self, n):
        return jax.random.permutation(self._next(), n)


kernel_name = 'concat_heads__sliding_block_cached__sliding_block_cached__decode'

def setup_inputs():
    _rng = _Rng(jax.random.key(int.from_bytes(__import__("os").urandom(4), "little")))
    _w = (lambda a: (lambda t: t.astype(jnp.bfloat16) if jnp.issubdtype(t.dtype, jnp.floating) else t)(jnp.asarray(a)))
    def _A_setup():
        B, Sq, D = 2, 1, 640
        Hq, Hkv, Sk, Dh = 32, 32, 4096, 128
        assert Hq % Hkv == 0, (Hq, Hkv)
        return {
            "x": _w((lambda *s: _rng.normal(s) * 0.8)(B, Sq, D)),
            "k_cache": _w((lambda *s: _rng.normal(s) * 0.8)(B, Hkv, Sk, Dh)),
            "v_cache": _w((lambda *s: _rng.normal(s) * 0.05)(B, Hkv, Sk, Dh)),
            "wq": _w((lambda *s: _rng.normal(s) * 0.8)(D, Hq * Dh) * (D ** -0.5)),
            "wo": _w((lambda *s: _rng.normal(s) * 0.05)(Hq * Dh, D) * ((Hq * Dh) ** -0.5)),
        }
    _A_in = _A_setup()

    def _B_setup():
        B, Sq, D = 2, 1, 640
        Hq, Hkv, Sk, Dh = 32, 32, 4096, 128
        assert Hq % Hkv == 0, (Hq, Hkv)
        return {
            "x": _w((lambda *s: _rng.normal(s) * 0.8)(B, Sq, D)),
            "k_cache": _w((lambda *s: _rng.normal(s) * 0.8)(B, Hkv, Sk, Dh)),
            "v_cache": _w((lambda *s: _rng.normal(s) * 0.05)(B, Hkv, Sk, Dh)),
            "wq": _w((lambda *s: _rng.normal(s) * 0.8)(D, Hq * Dh) * (D ** -0.5)),
            "wo": _w((lambda *s: _rng.normal(s) * 0.05)(Hq * Dh, D) * ((Hq * Dh) ** -0.5)),
        }
    _B_in = _B_setup()

    return {
        "A_x": _A_in["x"],
        "A_k_cache": _A_in["k_cache"],
        "A_v_cache": _A_in["v_cache"],
        "A_wq": _A_in["wq"],
        "A_wo": _A_in["wo"],
        "B_x": _B_in["x"],
        "B_k_cache": _B_in["k_cache"],
        "B_v_cache": _B_in["v_cache"],
        "B_wq": _B_in["wq"],
        "B_wo": _B_in["wo"],
    }

def reference(A_x, A_k_cache, A_v_cache, A_wq, A_wo, B_x, B_k_cache, B_v_cache, B_wq, B_wo):
    def _A_ref(x, k_cache, v_cache, wq, wo):
        B, Sq, D = x.shape
        Hq, Dh = 32, 128
        Hkv, Sk = k_cache.shape[1], k_cache.shape[2]
        W = min(4096, max(256, Sk // 4))
        rep = Hq // Hkv
        q = (lambda x, *d: x.transpose(*d))((x @ wq).reshape(B, Sq, Hq, Dh), 0, 2, 1, 3)
        k = jnp.repeat(k_cache[:, :, Sk - W:, :], rep, axis=1)
        v = jnp.repeat(v_cache[:, :, Sk - W:, :], rep, axis=1)
        scores = jnp.einsum("bhqd,bhkd->bhqk", q, k) * (Dh ** -0.5)
        p = _softmax(scores, axis=-1)
        o = jnp.einsum("bhqk,bhkd->bhqd", p, v)
        return (lambda x, *d: x.transpose(*d))(o, 0, 2, 1, 3).reshape(B, Sq, Hq * Dh) @ wo

    def _B_ref(x, k_cache, v_cache, wq, wo):
        B, Sq, D = x.shape
        Hq, Dh = 32, 128
        Hkv, Sk = k_cache.shape[1], k_cache.shape[2]
        W = min(4096, max(256, Sk // 4))
        rep = Hq // Hkv
        q = (lambda x, *d: x.transpose(*d))((x @ wq).reshape(B, Sq, Hq, Dh), 0, 2, 1, 3)
        k = jnp.repeat(k_cache[:, :, Sk - W:, :], rep, axis=1)
        v = jnp.repeat(v_cache[:, :, Sk - W:, :], rep, axis=1)
        scores = jnp.einsum("bhqd,bhkd->bhqk", q, k) * (Dh ** -0.5)
        p = _softmax(scores, axis=-1)
        o = jnp.einsum("bhqk,bhkd->bhqd", p, v)
        return (lambda x, *d: x.transpose(*d))(o, 0, 2, 1, 3).reshape(B, Sq, Hq * Dh) @ wo

    a = _A_ref(A_x, A_k_cache, A_v_cache, A_wq, A_wo)
    b = _B_ref(B_x, B_k_cache, B_v_cache, B_wq, B_wo)
    return jnp.concatenate([a, b], axis=-1)
```

```python
import jax
import jax.numpy as jnp
from jax import lax
from jax.experimental import pallas as pl
from jax.experimental.pallas import tpu as pltpu

B, D, H, SK, DH = 2, 640, 32, 4096, 128
W = min(4096, max(256, SK // 4))
OFF = SK - W
SCALE = float(DH) ** -0.5

DEPTH = 4
KV_ROWS = 128
NQ = 40
NO = 4


def _kv_pattern():
    npc = W // KV_ROWS
    hh = npc // 2
    order = []
    for s in range(hh):
        order += [(0, s, 0), (1, s + hh, 1), (1, s, 0), (0, s + hh, 1)]
    return order


def _kernel(ax, ak, av, awq, awo, bx, bk, bv, bwq, bwo, out_ref,
            xbuf, wqbuf, wobuf, kbuf, vbuf, outbuf, hsem, wosem, xsem, osem):
    xs, ks, vs, wqs, wos = (ax, bx), (ak, bk), (av, bv), (awq, bwq), (awo, bwo)
    pattern = _kv_pattern()

    def step_start(br, h, slot):
        copies = []
        r = D // NQ
        for s in range(NQ):
            copies.append((wqs[br].at[pl.ds(s * r, r), pl.ds(pl.multiple_of(h * DH, DH), DH)],
                           wqbuf.at[slot, pl.ds(s * r, r), :], hsem.at[slot], s % 2))
        for b in range(B):
            for a, s, p in pattern:
                copies.append((((ks, vs)[a][br]).at[b, h, pl.ds(OFF + s * KV_ROWS, KV_ROWS), :],
                               ((kbuf, vbuf)[a]).at[slot, b, pl.ds(s * KV_ROWS, KV_ROWS), :], hsem.at[slot], p))
        r = DH // NO
        for s in range(NO):
            copies.append((wos[br].at[pl.ds(pl.multiple_of(h * DH + s * r, r), r), :],
                           wobuf.at[slot, pl.ds(s * r, r), :], wosem.at[slot], s % 2))
        for src, dst, sem, p in copies:
            pltpu.make_async_copy(src, dst, sem).start(priority=p)

    def step_wait(slot):
        pltpu.make_async_copy(kbuf.at[slot], kbuf.at[slot], hsem.at[slot]).wait()
        pltpu.make_async_copy(vbuf.at[slot], vbuf.at[slot], hsem.at[slot]).wait()
        pltpu.make_async_copy(wqbuf.at[slot], wqbuf.at[slot], hsem.at[slot]).wait()

    row = lax.broadcasted_iota(jnp.int32, (B, 1), 0)
    nt = (((1,), (1,)), ((), ()))

    def head_compute(br, slot, acc):
        q = jnp.dot(xbuf[br], wqbuf[slot], preferred_element_type=jnp.float32).astype(jnp.bfloat16)
        s0 = lax.dot_general(q, kbuf[slot, 0], nt, preferred_element_type=jnp.float32)
        s1 = lax.dot_general(q, kbuf[slot, 1], nt, preferred_element_type=jnp.float32)
        s = jnp.where(row == 0, s0, s1) * SCALE
        m = jnp.max(s, axis=-1, keepdims=True)
        p = jnp.exp(s - m)
        l = jnp.sum(p, axis=-1, keepdims=True)
        pb = p.astype(jnp.bfloat16)
        o0 = jnp.dot(pb, vbuf[slot, 0], preferred_element_type=jnp.float32)
        o1 = jnp.dot(pb, vbuf[slot, 1], preferred_element_type=jnp.float32)
        o = (jnp.where(row == 0, o0, o1) / l).astype(jnp.bfloat16)
        pltpu.make_async_copy(wobuf.at[slot], wobuf.at[slot], wosem.at[slot]).wait()
        return acc + jnp.dot(o, wobuf[slot], preferred_element_type=jnp.float32)

    for br in range(2):
        pltpu.make_async_copy(xs[br], xbuf.at[br], xsem.at[br]).start()

    def loop(j, acc):
        slot = lax.rem(j, DEPTH)
        g = jnp.maximum(j - DEPTH, 0)
        br = lax.shift_right_logical(g, 5)
        h = lax.bitwise_and(g, H - 1)

        @pl.when(j == DEPTH)
        def _():
            for b_ in range(2):
                pltpu.make_async_copy(xs[b_], xbuf.at[b_], xsem.at[b_]).wait()

        def do(acc):
            step_wait(slot)
            acc = jnp.where(h == 0, jnp.zeros_like(acc), acc)
            acc = head_compute(br, slot, acc)

            @pl.when(h == H - 1)
            def _():
                outbuf[:, pl.ds(pl.multiple_of(br * D, 128), D)] = acc.astype(jnp.bfloat16)
            return acc

        acc = lax.cond(j >= DEPTH, do, lambda a: a, acc)

        @pl.when(j < H)
        def _():
            step_start(0, j, slot)

        @pl.when((j >= H) & (j < 2 * H))
        def _():
            step_start(1, j - H, slot)

        return acc

    lax.fori_loop(0, 2 * H + DEPTH, loop, jnp.zeros((B, D), jnp.float32))
    cp = pltpu.make_async_copy(outbuf, out_ref, osem.at[0])
    cp.start()
    cp.wait()


@jax.jit
def pallas_concat_heads__sliding_block_cached__sliding_block_cached__decode_kernel(
    A_x: jax.Array,
    A_k_cache: jax.Array,
    A_v_cache: jax.Array,
    A_wq: jax.Array,
    A_wo: jax.Array,
    B_x: jax.Array,
    B_k_cache: jax.Array,
    B_v_cache: jax.Array,
    B_wq: jax.Array,
    B_wo: jax.Array,
):
    any_ = pl.BlockSpec(memory_space=pl.ANY)
    out = pl.pallas_call(
        _kernel,
        out_shape=jax.ShapeDtypeStruct((B, 2 * D), jnp.bfloat16),
        in_specs=[any_] * 10,
        out_specs=any_,
        scratch_shapes=[
            pltpu.VMEM((2, B, D), jnp.bfloat16),
            pltpu.VMEM((DEPTH, D, DH), jnp.bfloat16),
            pltpu.VMEM((DEPTH, DH, D), jnp.bfloat16),
            pltpu.VMEM((DEPTH, B, W, DH), jnp.bfloat16),
            pltpu.VMEM((DEPTH, B, W, DH), jnp.bfloat16),
            pltpu.VMEM((B, 2 * D), jnp.bfloat16),
            pltpu.SemaphoreType.DMA((DEPTH,)),
            pltpu.SemaphoreType.DMA((DEPTH,)),
            pltpu.SemaphoreType.DMA((2,)),
            pltpu.SemaphoreType.DMA((1,)),
        ],
        compiler_params=pltpu.CompilerParams(
            vmem_limit_bytes=64 * 1024 * 1024,
            disable_semaphore_checks=True,
            disable_bounds_checks=True,
        ),
    )(A_x.reshape(B, D), A_k_cache, A_v_cache, A_wq, A_wo,
      B_x.reshape(B, D), B_k_cache, B_v_cache, B_wq, B_wo)
    return out.reshape(B, 1, 2 * D)
```

```python
import jax
import jax.numpy as jnp
from jax import lax
from jax.experimental import pallas as pl
from jax.experimental.pallas import tpu as pltpu

B, D, H, SK, DH = 2, 640, 32, 4096, 128
W = min(4096, max(256, SK // 4))
OFF = SK - W
SCALE = float(DH) ** -0.5
NSTEP = 2 * H

DEPTH = 4
KV_ROWS = 128
WQ_ROWS = 16
WQ_COLS = 1024
WQ_BLOCKS = D // WQ_ROWS
NT = (((1,), (1,)), ((), ()))


def _kernel(ax, ak, av, awq, awo, bx, bk, bv, bwq, bwo, out_ref,
            xbuf, wqbuf, wobuf, kbuf, vbuf, outbuf, ksem, vsem, wosem, xsem, osem, qsem):
    xs, ks, vs, wqs, wos = (ax, bx), (ak, bk), (av, bv), (awq, bwq), (awo, bwo)

    def wq_start(br, i):
        for blk, p0 in ((i, 0), (i + WQ_BLOCKS // 2, 1)):
            r0 = pl.multiple_of(blk * WQ_ROWS, WQ_ROWS)
            for c in range(H * DH // WQ_COLS):
                pltpu.make_async_copy(
                    wqs[br].at[pl.ds(r0, WQ_ROWS), pl.ds(c * WQ_COLS, WQ_COLS)],
                    wqbuf.at[br, pl.ds(r0, WQ_ROWS), pl.ds(c * WQ_COLS, WQ_COLS)],
                    qsem.at[br]).start(priority=(p0 + c) % 2)

    def kv_start(br, h, slot):
        for s in range(W // KV_ROWS):
            for b in range(B):
                src = pl.ds(OFF + s * KV_ROWS, KV_ROWS)
                dst = pl.ds(s * KV_ROWS, KV_ROWS)
                pltpu.make_async_copy(ks[br].at[b, h, src, :], kbuf.at[slot, b, dst, :],
                                      ksem.at[slot]).start(priority=0)
                pltpu.make_async_copy(vs[br].at[b, h, src, :], vbuf.at[slot, b, dst, :],
                                      vsem.at[B * slot + b]).start(priority=1)
        if br == 0:
            @pl.when(h < WQ_BLOCKS // 2)
            def _():
                wq_start(1, h)

    def wo_start(br, h, slot):
        pltpu.make_async_copy(wos[br].at[pl.ds(pl.multiple_of(h * DH, DH), DH), :], wobuf.at[slot],
                              wosem.at[slot]).start(priority=1)

    row = lax.broadcasted_iota(jnp.int32, (B, 1), 0)

    def ld(buf, slot, b):
        return pltpu.bitcast(buf.bitcast(jnp.uint32)[slot, b], jnp.bfloat16)

    def stage_a(g):
        br = lax.shift_right_logical(g, 5)
        h = lax.bitwise_and(g, H - 1)
        slot = lax.rem(g, DEPTH)

        @pl.when(h == 0)
        def _():
            pltpu.make_async_copy(wqbuf.at[br], wqbuf.at[br], qsem.at[br]).wait()

        wq_h = wqbuf[br, :, pl.ds(pl.multiple_of(h * DH, DH), DH)]
        q = jnp.dot(xbuf[br], wq_h, preferred_element_type=jnp.float32).astype(jnp.bfloat16)
        pltpu.make_async_copy(kbuf.at[slot], kbuf.at[slot], ksem.at[slot]).wait()
        s0 = lax.dot_general(q, ld(kbuf, slot, 0), NT, preferred_element_type=jnp.float32)
        s1 = lax.dot_general(q, ld(kbuf, slot, 1), NT, preferred_element_type=jnp.float32)
        s = jnp.where(row == 0, s0, s1) * SCALE
        m = jnp.max(s, axis=-1, keepdims=True)
        p = jnp.exp(s - m)
        l = jnp.sum(p, axis=-1, keepdims=True)
        return p.astype(jnp.bfloat16), l

    def stage_b(g, pb, l):
        slot = lax.rem(g, DEPTH)
        pltpu.make_async_copy(vbuf.at[slot, 0], vbuf.at[slot, 0], vsem.at[B * slot]).wait()
        o0 = jnp.dot(pb, ld(vbuf, slot, 0), preferred_element_type=jnp.float32)
        pltpu.make_async_copy(vbuf.at[slot, 1], vbuf.at[slot, 1], vsem.at[B * slot + 1]).wait()
        o1 = jnp.dot(pb, ld(vbuf, slot, 1), preferred_element_type=jnp.float32)
        return (jnp.where(row == 0, o0, o1) / l).astype(jnp.bfloat16)

    def stage_c(g, o, acc):
        br = lax.shift_right_logical(g, 5)
        h = lax.bitwise_and(g, H - 1)
        slot = lax.rem(g, DEPTH)
        pltpu.make_async_copy(wobuf.at[slot], wobuf.at[slot], wosem.at[slot]).wait()
        acc = jnp.where(h == 0, jnp.zeros_like(acc), acc)
        acc = acc + jnp.dot(o, wobuf[slot], preferred_element_type=jnp.float32)

        @pl.when(h == H - 1)
        def _():
            outbuf[:, pl.ds(pl.multiple_of(br * D, 128), D)] = acc.astype(jnp.bfloat16)
        return acc

    for br in range(2):
        pltpu.make_async_copy(xs[br], xbuf.at[br], xsem.at[br]).start()

    def wq_a(i, carry):
        wq_start(0, i)
        return carry

    lax.fori_loop(0, WQ_BLOCKS // 2, wq_a, 0)

    def loop(n, carry):
        pb, l, o, acc = carry
        i = n - DEPTH

        @pl.when(i == 0)
        def _():
            for br in range(2):
                pltpu.make_async_copy(xs[br], xbuf.at[br], xsem.at[br]).wait()

        npb, nl = lax.cond((i >= 0) & (i < NSTEP),
                           lambda: stage_a(jnp.maximum(i, 0)), lambda: (pb, l))
        no = lax.cond((i >= 1) & (i < NSTEP + 1),
                      lambda: stage_b(jnp.maximum(i - 1, 0), pb, l), lambda: o)
        nacc = lax.cond((i >= 2) & (i < NSTEP + 2),
                        lambda: stage_c(jnp.maximum(i - 2, 0), o, acc), lambda: acc)

        j = n - 1
        slot = lax.rem(j, DEPTH)

        @pl.when(j < H)
        def _():
            kv_start(0, j, slot)

        @pl.when((j >= H) & (j < NSTEP))
        def _():
            kv_start(1, j - H, slot)

        jo = n - 2

        @pl.when((jo >= 0) & (jo < H))
        def _():
            wo_start(0, jnp.maximum(jo, 0), lax.rem(jo + DEPTH, DEPTH))

        @pl.when((jo >= H) & (jo < NSTEP))
        def _():
            wo_start(1, jo - H, lax.rem(jo + DEPTH, DEPTH))

        return npb, nl, no, nacc

    init = (jnp.zeros((B, W), jnp.bfloat16), jnp.ones((B, 1), jnp.float32),
            jnp.zeros((B, DH), jnp.bfloat16), jnp.zeros((B, D), jnp.float32))
    lax.fori_loop(1, NSTEP + DEPTH + 2, loop, init)

    cp = pltpu.make_async_copy(outbuf, out_ref, osem.at[0])
    cp.start()
    cp.wait()


@jax.jit
def pallas_concat_heads__sliding_block_cached__sliding_block_cached__decode_kernel(
    A_x: jax.Array,
    A_k_cache: jax.Array,
    A_v_cache: jax.Array,
    A_wq: jax.Array,
    A_wo: jax.Array,
    B_x: jax.Array,
    B_k_cache: jax.Array,
    B_v_cache: jax.Array,
    B_wq: jax.Array,
    B_wo: jax.Array,
):
    any_ = pl.BlockSpec(memory_space=pl.ANY)
    out = pl.pallas_call(
        _kernel,
        out_shape=jax.ShapeDtypeStruct((B, 2 * D), jnp.bfloat16),
        in_specs=[any_] * 10,
        out_specs=any_,
        scratch_shapes=[
            pltpu.VMEM((2, B, D), jnp.bfloat16),
            pltpu.VMEM((2, D, H * DH), jnp.bfloat16),
            pltpu.VMEM((DEPTH, DH, D), jnp.bfloat16),
            pltpu.VMEM((DEPTH, B, W, DH), jnp.bfloat16),
            pltpu.VMEM((DEPTH, B, W, DH), jnp.bfloat16),
            pltpu.VMEM((B, 2 * D), jnp.bfloat16),
            pltpu.SemaphoreType.DMA((DEPTH,)),
            pltpu.SemaphoreType.DMA((B * DEPTH,)),
            pltpu.SemaphoreType.DMA((DEPTH,)),
            pltpu.SemaphoreType.DMA((2,)),
            pltpu.SemaphoreType.DMA((1,)),
            pltpu.SemaphoreType.DMA((2,)),
        ],
        compiler_params=pltpu.CompilerParams(
            vmem_limit_bytes=64 * 1024 * 1024,
            disable_semaphore_checks=True,
            disable_bounds_checks=True,
        ),
    )(A_x.reshape(B, D), A_k_cache, A_v_cache, A_wq, A_wo,
      B_x.reshape(B, D), B_k_cache, B_v_cache, B_wq, B_wo)
    return out.reshape(B, 1, 2 * D)
```

```python
import jax
import jax.numpy as jnp
from jax import lax
from jax.experimental import pallas as pl
from jax.experimental.pallas import tpu as pltpu

B, D, H, SK, DH = 2, 640, 32, 4096, 128
W = min(4096, max(256, SK // 4))
OFF = SK - W
SCALE = float(DH) ** -0.5
NSTEP = 2 * H

DEPTH = 4
KV_ROWS = 128
WQ_ROWS = 16
WQ_COLS = 1024
WQ_BLOCKS = D // WQ_ROWS
NT = (((1,), (1,)), ((), ()))


def _kernel(ax, ak, av, awq, awo, bx, bk, bv, bwq, bwo, out_ref,
            xbuf, wqbuf, wobuf, kbuf, vbuf, outbuf, ksem, vsem, wosem, xsem, osem, qsem):
    xs, ks, vs, wqs, wos = (ax, bx), (ak, bk), (av, bv), (awq, bwq), (awo, bwo)

    def wq_start(br, i):
        for blk, p0 in ((i, 0), (i + WQ_BLOCKS // 2, 1)):
            r0 = pl.multiple_of(blk * WQ_ROWS, WQ_ROWS)
            for c in range(H * DH // WQ_COLS):
                pltpu.make_async_copy(
                    wqs[br].at[pl.ds(r0, WQ_ROWS), pl.ds(c * WQ_COLS, WQ_COLS)],
                    wqbuf.at[br, pl.ds(r0, WQ_ROWS), pl.ds(c * WQ_COLS, WQ_COLS)],
                    qsem.at[br]).start(priority=(p0 + c) % 2)

    def kv_start(br, h, slot):
        for s in range(W // KV_ROWS):
            for b in range(B):
                src = pl.ds(OFF + s * KV_ROWS, KV_ROWS)
                dst = pl.ds(s * KV_ROWS, KV_ROWS)
                pltpu.make_async_copy(ks[br].at[b, h, src, :], kbuf.at[slot, b, dst, :],
                                      ksem.at[slot]).start(priority=0)
                pltpu.make_async_copy(vs[br].at[b, h, src, :], vbuf.at[slot, b, dst, :],
                                      vsem.at[B * slot + b]).start(priority=1)
        if br == 0:
            @pl.when(h < WQ_BLOCKS // 2)
            def _():
                wq_start(1, h)

    def wo_start(br, h, slot):
        pltpu.make_async_copy(wos[br].at[pl.ds(pl.multiple_of(h * DH, DH), DH), :], wobuf.at[slot],
                              wosem.at[slot]).start(priority=1)

    row = lax.broadcasted_iota(jnp.int32, (B, 1), 0)

    def stage_a(g):
        br = lax.shift_right_logical(g, 5)
        h = lax.bitwise_and(g, H - 1)
        slot = lax.rem(g, DEPTH)

        @pl.when(h == 0)
        def _():
            pltpu.make_async_copy(wqbuf.at[br], wqbuf.at[br], qsem.at[br]).wait()

        wq_h = wqbuf[br, :, pl.ds(pl.multiple_of(h * DH, DH), DH)]
        q = jnp.dot(xbuf[br], wq_h, preferred_element_type=jnp.float32).astype(jnp.bfloat16)
        pltpu.make_async_copy(kbuf.at[slot], kbuf.at[slot], ksem.at[slot]).wait()
        s0 = lax.dot_general(q, kbuf[slot, 0], NT, preferred_element_type=jnp.float32)
        s1 = lax.dot_general(q, kbuf[slot, 1], NT, preferred_element_type=jnp.float32)
        s = jnp.where(row == 0, s0, s1) * SCALE
        m = jnp.max(s, axis=-1, keepdims=True)
        p = jnp.exp(s - m)
        l = jnp.sum(p, axis=-1, keepdims=True)
        return p.astype(jnp.bfloat16), l

    def stage_b(g, pb, l):
        slot = lax.rem(g, DEPTH)
        pltpu.make_async_copy(vbuf.at[slot, 0], vbuf.at[slot, 0], vsem.at[B * slot]).wait()
        o0 = jnp.dot(pb, vbuf[slot, 0], preferred_element_type=jnp.float32)
        pltpu.make_async_copy(vbuf.at[slot, 1], vbuf.at[slot, 1], vsem.at[B * slot + 1]).wait()
        o1 = jnp.dot(pb, vbuf[slot, 1], preferred_element_type=jnp.float32)
        return (jnp.where(row == 0, o0, o1) / l).astype(jnp.bfloat16)

    def stage_c(g, o, acc):
        br = lax.shift_right_logical(g, 5)
        h = lax.bitwise_and(g, H - 1)
        slot = lax.rem(g, DEPTH)
        pltpu.make_async_copy(wobuf.at[slot], wobuf.at[slot], wosem.at[slot]).wait()
        acc = jnp.where(h == 0, jnp.zeros_like(acc), acc)
        acc = acc + jnp.dot(o, wobuf[slot], preferred_element_type=jnp.float32)

        @pl.when(h == H - 1)
        def _():
            outbuf[:, pl.ds(pl.multiple_of(br * D, 128), D)] = acc.astype(jnp.bfloat16)
        return acc

    for br in range(2):
        pltpu.make_async_copy(xs[br], xbuf.at[br], xsem.at[br]).start()

    def wq_a(i, carry):
        wq_start(0, i)
        return carry

    lax.fori_loop(0, WQ_BLOCKS // 2, wq_a, 0)

    def loop(n, carry):
        pb, l, o, acc = carry
        i = n - DEPTH

        @pl.when(i == 0)
        def _():
            for br in range(2):
                pltpu.make_async_copy(xs[br], xbuf.at[br], xsem.at[br]).wait()

        npb, nl = lax.cond((i >= 0) & (i < NSTEP),
                           lambda: stage_a(jnp.maximum(i, 0)), lambda: (pb, l))
        no = lax.cond((i >= 1) & (i < NSTEP + 1),
                      lambda: stage_b(jnp.maximum(i - 1, 0), pb, l), lambda: o)
        nacc = lax.cond((i >= 2) & (i < NSTEP + 2),
                        lambda: stage_c(jnp.maximum(i - 2, 0), o, acc), lambda: acc)

        j = n - 1
        slot = lax.rem(j, DEPTH)

        @pl.when(j < H)
        def _():
            kv_start(0, j, slot)

        @pl.when((j >= H) & (j < NSTEP))
        def _():
            kv_start(1, j - H, slot)

        jo = n - 2

        @pl.when((jo >= 0) & (jo < H))
        def _():
            wo_start(0, jnp.maximum(jo, 0), lax.rem(jo + DEPTH, DEPTH))

        @pl.when((jo >= H) & (jo < NSTEP))
        def _():
            wo_start(1, jo - H, lax.rem(jo + DEPTH, DEPTH))

        return npb, nl, no, nacc

    init = (jnp.zeros((B, W), jnp.bfloat16), jnp.ones((B, 1), jnp.float32),
            jnp.zeros((B, DH), jnp.bfloat16), jnp.zeros((B, D), jnp.float32))
    lax.fori_loop(1, NSTEP + DEPTH + 2, loop, init)

    cp = pltpu.make_async_copy(outbuf, out_ref, osem.at[0])
    cp.start()
    cp.wait()


@jax.jit
def pallas_concat_heads__sliding_block_cached__sliding_block_cached__decode_kernel(
    A_x: jax.Array,
    A_k_cache: jax.Array,
    A_v_cache: jax.Array,
    A_wq: jax.Array,
    A_wo: jax.Array,
    B_x: jax.Array,
    B_k_cache: jax.Array,
    B_v_cache: jax.Array,
    B_wq: jax.Array,
    B_wo: jax.Array,
):
    any_ = pl.BlockSpec(memory_space=pl.ANY)
    out = pl.pallas_call(
        _kernel,
        out_shape=jax.ShapeDtypeStruct((B, 2 * D), jnp.bfloat16),
        in_specs=[any_] * 10,
        out_specs=any_,
        scratch_shapes=[
            pltpu.VMEM((2, B, D), jnp.bfloat16),
            pltpu.VMEM((2, D, H * DH), jnp.bfloat16),
            pltpu.VMEM((DEPTH, DH, D), jnp.bfloat16),
            pltpu.VMEM((DEPTH, B, W, DH), jnp.bfloat16),
            pltpu.VMEM((DEPTH, B, W, DH), jnp.bfloat16),
            pltpu.VMEM((B, 2 * D), jnp.bfloat16),
            pltpu.SemaphoreType.DMA((DEPTH,)),
            pltpu.SemaphoreType.DMA((B * DEPTH,)),
            pltpu.SemaphoreType.DMA((DEPTH,)),
            pltpu.SemaphoreType.DMA((2,)),
            pltpu.SemaphoreType.DMA((1,)),
            pltpu.SemaphoreType.DMA((2,)),
        ],
        compiler_params=pltpu.CompilerParams(
            vmem_limit_bytes=64 * 1024 * 1024,
            disable_semaphore_checks=True,
            disable_bounds_checks=True,
        ),
    )(A_x.reshape(B, D), A_k_cache, A_v_cache, A_wq, A_wo,
      B_x.reshape(B, D), B_k_cache, B_v_cache, B_wq, B_wo)
    return out.reshape(B, 1, 2 * D)
```
